```python
import jax
import jax.numpy as jnp

def _softmax(x, axis=-1):
    return jax.nn.softmax(x, axis=axis)
def _gelu(x):
    return jax.nn.gelu(x, approximate=True)
def _silu(x):
    return jax.nn.silu(x)
def _sigmoid(x):
    return jax.nn.sigmoid(x)
def _layernorm(x, axis=-1, eps=1e-5):
    m = jnp.mean(x, axis=axis, keepdims=True)
    v = jnp.var(x, axis=axis, keepdims=True)
    return (x - m) / jnp.sqrt(v + eps)
def _scatter_add(tgt, idx, src, axis=0):
    return tgt.at[idx].add(src)
def _segment_sum(src, seg, n):
    return jax.ops.segment_sum(src, seg, n)
class _Rng:
    def __init__(self, key):
        self._k = key
    def _next(self):
        self._k, sub = jax.random.split(self._k)
        return sub
    def normal(self, shape):
        return jax.random.normal(self._next(), shape, dtype=jnp.bfloat16)
    def randint(self, lo, hi, shape):
        return jax.random.randint(self._next(), shape, lo, hi, dtype=jnp.int32)
    def uniform(self, shape, lo=0.0, hi=1.0):
        return jax.random.uniform(self._next(), shape, jnp.bfloat16, lo, hi)
    def permutation(self, n):
        return jax.random.permutation(self._next(), n)


kernel_name = 'parallel_sum__sliding_block_cached__glu_gated_swiglu__decode'

def setup_inputs():
    _rng = _Rng(jax.random.key(int.from_bytes(__import__("os").urandom(4), "little")))
    _w = (lambda a: (lambda t: t.astype(jnp.bfloat16) if jnp.issubdtype(t.dtype, jnp.floating) else t)(jnp.asarray(a)))
    def _A_setup():
        B, Sq, D = 4, 1, 640
        Hq, Hkv, Sk, Dh = 32, 32, 8192, 192
        assert Hq % Hkv == 0, (Hq, Hkv)
        return {
            "x": _w((lambda *s: _rng.normal(s) * 0.05)(B, Sq, D)),
            "k_cache": _w((lambda *s: _rng.normal(s) * 0.05)(B, Hkv, Sk, Dh)),
            "v_cache": _w((lambda *s: _rng.normal(s) * 0.05)(B, Hkv, Sk, Dh)),
            "wq": _w((lambda *s: _rng.normal(s) * 0.05)(D, Hq * Dh) * (D ** -0.5)),
            "wo": _w((lambda *s: _rng.normal(s) * 0.05)(Hq * Dh, D) * ((Hq * Dh) ** -0.5)),
        }
    _A_in = _A_setup()

    def _B_setup():
        B, S, D, F = 4, 1, 640, 1536
        return {
            "x": _w((lambda *s: _rng.normal(s) * 0.05)(B, S, D)),
            "w1": _w((lambda *s: _rng.normal(s) * 0.05)(D, F) * (2.0 / D) ** 0.5),
            "w3": _w((lambda *s: _rng.normal(s) * 0.05)(D, F) * (2.0 / D) ** 0.5),
            "w2": _w((lambda *s: _rng.normal(s) * 0.05)(F, D) * (2.0 / F) ** 0.5),
        }
    _B_in = _B_setup()

    return {
        "A_x": _A_in["x"],
        "A_k_cache": _A_in["k_cache"],
        "A_v_cache": _A_in["v_cache"],
        "A_wq": _A_in["wq"],
        "A_wo": _A_in["wo"],
        "B_x": _B_in["x"],
        "B_w1": _B_in["w1"],
        "B_w3": _B_in["w3"],
        "B_w2": _B_in["w2"],
    }

def reference(A_x, A_k_cache, A_v_cache, A_wq, A_wo, B_x, B_w1, B_w3, B_w2):
    def _A_ref(x, k_cache, v_cache, wq, wo):
        B, Sq, D = x.shape
        Hq, Dh = 32, 192
        Hkv, Sk = k_cache.shape[1], k_cache.shape[2]
        W = min(4096, max(256, Sk // 4))
        rep = Hq // Hkv
        q = (lambda x, *d: x.transpose(*d))((x @ wq).reshape(B, Sq, Hq, Dh), 0, 2, 1, 3)
        k = jnp.repeat(k_cache[:, :, Sk - W:, :], rep, axis=1)
        v = jnp.repeat(v_cache[:, :, Sk - W:, :], rep, axis=1)
        scores = jnp.einsum("bhqd,bhkd->bhqk", q, k) * (Dh ** -0.5)
        p = _softmax(scores, axis=-1)
        o = jnp.einsum("bhqk,bhkd->bhqd", p, v)
        return (lambda x, *d: x.transpose(*d))(o, 0, 2, 1, 3).reshape(B, Sq, Hq * Dh) @ wo

    def _B_ref(x, w1, w3, w2):
        gate = jnp.einsum("bsd,df->bsf", x, w1)
        up = jnp.einsum("bsd,df->bsf", x, w3)
        h = _silu(gate) * up
        out = jnp.einsum("bsf,fd->bsd", h, w2)
        return out

    x = A_x
    xn = _layernorm(x, axis=-1)
    return x + _A_ref(xn, A_k_cache, A_v_cache, A_wq, A_wo) + _B_ref(xn, B_w1, B_w3, B_w2)
```

```python
import functools

import jax
import jax.numpy as jnp
from jax import lax
import jax.experimental.pallas as pl
import jax.experimental.pallas.tpu as pltpu

_HQ = 32
_DH = 192
_EPS = 1e-5
_NBUF = 3
_NW2 = 4


def _kernel(x_hbm, k_hbm, v_hbm, wq_hbm, wo_hbm, w1_hbm, w3_hbm, w2_hbm,
            o_ref,
            x_v, wq_v, wo_v, w1_v, w3_v, w2_v, kbuf, vbuf, q_s,
            wsem, w2sem, ksem, vsem,
            *, B, D, F, Sk, W):
    H, Dh = _HQ, _DH
    f32, bf16 = jnp.float32, jnp.bfloat16
    scale = Dh ** -0.5
    w2_rows = F // _NW2

    def k_copy(h, b, slot):
        return pltpu.make_async_copy(
            k_hbm.at[b, h, :, pl.ds(Sk - W, W)], kbuf.at[slot, b], ksem.at[slot, b])

    def v_copy(h, b, slot):
        return pltpu.make_async_copy(
            v_hbm.at[b, h, :, pl.ds(Sk - W, W)], vbuf.at[slot, b], vsem.at[slot, b])

    def w2_copy(j):
        return pltpu.make_async_copy(
            w2_hbm.at[pl.ds(j * w2_rows, w2_rows)],
            w2_v.at[pl.ds(j * w2_rows, w2_rows)], w2sem.at[j])

    x_cp = pltpu.make_async_copy(x_hbm, x_v, wsem.at[0])
    wq_cp = pltpu.make_async_copy(wq_hbm, wq_v, wsem.at[1])
    wo_cp = pltpu.make_async_copy(wo_hbm, wo_v, wsem.at[2])
    w1_cp = pltpu.make_async_copy(w1_hbm, w1_v, wsem.at[3])
    w3_cp = pltpu.make_async_copy(w3_hbm, w3_v, wsem.at[4])

    def start_head(h, slot):
        for b in range(B):
            k_copy(h, b, slot).start()
        for b in range(B):
            v_copy(h, b, slot).start()

    x_cp.start()
    wq_cp.start()
    w1_cp.start()
    w3_cp.start()
    wo_cp.start()
    for s in range(_NBUF):
        start_head(s, s)

    x_cp.wait()
    x = x_v[...].astype(f32)
    mu = jnp.mean(x, axis=-1, keepdims=True)
    xc = x - mu
    var = jnp.mean(xc * xc, axis=-1, keepdims=True)
    xn = (xc / jnp.sqrt(var + _EPS)).astype(bf16)

    wq_cp.wait()
    q_all = jnp.dot(xn, wq_v[...], preferred_element_type=f32)
    for h in range(H):
        q_s[h] = q_all[:, h * Dh:(h + 1) * Dh]

    w1_cp.wait()
    w3_cp.wait()
    gate = jnp.dot(xn, w1_v[...], preferred_element_type=f32)
    up = jnp.dot(xn, w3_v[...], preferred_element_type=f32)
    hid = (gate * jax.nn.sigmoid(gate) * up).astype(bf16)
    wo_cp.wait()

    row = lax.broadcasted_iota(jnp.int32, (B, 1), 0)

    def head_step(h, acc):
        slot = lax.rem(h, _NBUF)
        q = q_s[h].astype(bf16)
        s = None
        for b in range(B):
            k_copy(h, b, slot).wait()
            sb = jnp.dot(q, kbuf[slot, b], preferred_element_type=f32)
            s = sb if s is None else jnp.where(row == b, sb, s)
        s = s * scale
        m = jnp.max(s, axis=-1, keepdims=True)
        p = jnp.exp(s - m).astype(bf16)
        l = jnp.sum(p.astype(f32), axis=-1, keepdims=True)
        o = None
        for b in range(B):
            v_copy(h, b, slot).wait()
            ob = lax.dot_general(p, vbuf[slot, b], (((1,), (1,)), ((), ())),
                                 preferred_element_type=f32)
            o = ob if o is None else jnp.where(row == b, ob, o)
        o = (o / l).astype(bf16)
        r0 = pl.multiple_of(h * Dh, 16)
        acc = acc + jnp.dot(o, wo_v[pl.ds(r0, Dh), :], preferred_element_type=f32)

        @pl.when(h + _NBUF < H)
        def _():
            start_head(h + _NBUF, slot)

        @pl.when(h + _NBUF == H)
        def _():
            for j in range(_NW2):
                w2_copy(j).start()

        return acc

    acc = lax.fori_loop(0, H, head_step, x)

    for j in range(_NW2):
        w2_copy(j).wait()
        acc = acc + jnp.dot(hid[:, j * w2_rows:(j + 1) * w2_rows],
                            w2_v[j * w2_rows:(j + 1) * w2_rows, :],
                            preferred_element_type=f32)
    o_ref[...] = acc.astype(o_ref.dtype)


@jax.jit
def pallas_parallel_sum__sliding_block_cached__glu_gated_swiglu__decode_kernel(
    A_x: jax.Array,
    A_k_cache: jax.Array,
    A_v_cache: jax.Array,
    A_wq: jax.Array,
    A_wo: jax.Array,
    B_x: jax.Array,
    B_w1: jax.Array,
    B_w3: jax.Array,
    B_w2: jax.Array,
):
    B, Sq, D = A_x.shape
    _, Hkv, Sk, Dh = A_k_cache.shape
    F = B_w1.shape[1]
    assert Sq == 1 and Hkv == _HQ and Dh == _DH
    W = min(4096, max(256, Sk // 4))
    bf16 = jnp.bfloat16

    kt = jnp.swapaxes(A_k_cache, 2, 3)
    vt = jnp.swapaxes(A_v_cache, 2, 3)
    x2 = A_x.reshape(B, D)

    any_spec = pl.BlockSpec(memory_space=pl.ANY)
    out = pl.pallas_call(
        functools.partial(_kernel, B=B, D=D, F=F, Sk=Sk, W=W),
        in_specs=[any_spec] * 8,
        out_specs=pl.BlockSpec(memory_space=pltpu.VMEM),
        out_shape=jax.ShapeDtypeStruct((B, D), A_x.dtype),
        scratch_shapes=[
            pltpu.VMEM((B, D), bf16),
            pltpu.VMEM(A_wq.shape, bf16),
            pltpu.VMEM(A_wo.shape, bf16),
            pltpu.VMEM(B_w1.shape, bf16),
            pltpu.VMEM(B_w3.shape, bf16),
            pltpu.VMEM(B_w2.shape, bf16),
            pltpu.VMEM((_NBUF, B, _DH, W), bf16),
            pltpu.VMEM((_NBUF, B, _DH, W), bf16),
            pltpu.VMEM((_HQ, B, _DH), jnp.float32),
            pltpu.SemaphoreType.DMA((5,)),
            pltpu.SemaphoreType.DMA((_NW2,)),
            pltpu.SemaphoreType.DMA((_NBUF, B)),
            pltpu.SemaphoreType.DMA((_NBUF, B)),
        ],
        compiler_params=pltpu.CompilerParams(vmem_limit_bytes=100 * 1024 * 1024),
    )(x2, kt, vt, A_wq, A_wo, B_w1, B_w3, B_w2)
    return out.reshape(B, Sq, D)
```

```python
import functools

import jax
import jax.numpy as jnp
from jax import lax
import jax.experimental.pallas as pl
import jax.experimental.pallas.tpu as pltpu

_HQ = 32
_DH = 192
_EPS = 1e-5
_LANES = 128
_W2_GROUPS = (10, 8, 4, 2)
_WO_ROWS = 64


def _kernel(x_hbm, k_hbm, v_hbm, wq_hbm, wo_hbm, w1_hbm, w3_hbm, w2_hbm,
            o_ref,
            x_v, wq_v, wo_v, w1_v, w3_v, w2_v, kbuf, vbuf, q_s,
            wsem, w2sem, ksem, vsem,
            *, B, D, F, Sk, W):
    H, Dh = _HQ, _DH
    HP = H // 2
    R = 2 * Dh
    NC = W // _LANES
    f32, bf16 = jnp.float32, jnp.bfloat16
    scale = Dh ** -0.5

    def start_unit(hp, b):
        r0 = pl.multiple_of((b * HP + hp) * R, R)
        for c in range(NC):
            cols = pl.ds(Sk - W + c * _LANES, _LANES)
            pltpu.make_async_copy(k_hbm.at[pl.ds(r0, R), cols], kbuf.at[b, c],
                                  ksem.at[b]).start(priority=0)
            pltpu.make_async_copy(v_hbm.at[pl.ds(r0, R), cols], vbuf.at[b, c],
                                  vsem.at[b]).start(priority=1)

    def wait_all(buf, sem):
        pltpu.make_async_copy(buf, buf, sem).wait()

    def start_rows(src, dst, sem, rows, first, count):
        def body(i, carry):
            for p in range(2):
                r = pl.multiple_of((first + 2 * i + p) * rows, 8)
                pltpu.make_async_copy(src.at[pl.ds(r, rows)], dst.at[pl.ds(r, rows)],
                                      sem).start(priority=p)
            return carry
        lax.fori_loop(0, count // 2, body, 0)

    x_cp = pltpu.make_async_copy(x_hbm, x_v, wsem.at[0])
    x_cp.start()
    start_rows(wq_hbm, wq_v, wsem.at[1], 8, 0, D // 8)
    start_rows(w1_hbm, w1_v, wsem.at[3], 32, 0, D // 32)
    start_rows(w3_hbm, w3_v, wsem.at[4], 32, 0, D // 32)
    start_rows(wo_hbm, wo_v, wsem.at[2], _WO_ROWS, 0, H * Dh // _WO_ROWS)
    for b in range(B):
        start_unit(0, b)

    x_cp.wait()
    x = x_v[...].astype(f32)
    mu = jnp.mean(x, axis=-1, keepdims=True)
    xc = x - mu
    var = jnp.mean(xc * xc, axis=-1, keepdims=True)
    xn = xc / jnp.sqrt(var + _EPS)
    xn2 = jnp.concatenate([xn, xn], axis=0).astype(bf16)

    row = lax.broadcasted_iota(jnp.int32, (2 * B, R), 0)
    col = lax.broadcasted_iota(jnp.int32, (2 * B, R), 1)
    diag = (row >= B) == (col >= Dh)
    row_b = jnp.where(row >= B, row - B, row)

    wait_all(wq_v, wsem.at[1])
    for hp in range(HP):
        q = jnp.dot(xn2, wq_v[:, hp * R:(hp + 1) * R], preferred_element_type=f32)
        q_s[hp] = jnp.where(diag, q, 0.0)

    wait_all(w1_v, wsem.at[3])
    wait_all(w3_v, wsem.at[4])
    gate = jnp.dot(xn2, w1_v[...], preferred_element_type=f32)
    up = jnp.dot(xn2, w3_v[...], preferred_element_type=f32)
    hid = (gate * jax.nn.sigmoid(gate) * up).astype(bf16)
    wait_all(wo_v, wsem.at[2])

    def pair_step(hp, acc):
        q = q_s[hp].astype(bf16)
        o_sel = jnp.zeros((2 * B, R), f32)
        for b in range(B):
            wait_all(kbuf.at[b], ksem.at[b])
            s = [jnp.dot(q, kbuf[b, c], preferred_element_type=f32) * scale
                 for c in range(NC)]
            m = functools.reduce(jnp.maximum, s)
            m = jnp.max(m, axis=-1, keepdims=True)
            p = [jnp.exp(sc - m).astype(bf16) for sc in s]
            l = functools.reduce(jnp.add, [pc.astype(f32) for pc in p])
            l = jnp.sum(l, axis=-1, keepdims=True)
            wait_all(vbuf.at[b], vsem.at[b])
            o = functools.reduce(jnp.add, [
                lax.dot_general(p[c], vbuf[b, c], (((1,), (1,)), ((), ())),
                                preferred_element_type=f32)
                for c in range(NC)])
            o_sel = jnp.where(row_b == b, o / l, o_sel)

            @pl.when(hp + 1 < HP)
            def _():
                start_unit(hp + 1, b)

            if b == 0:
                @pl.when(hp + 1 == HP)
                def _():
                    first = 0
                    for g, n in enumerate(_W2_GROUPS):
                        start_rows(w2_hbm, w2_v, w2sem.at[g], _WO_ROWS, first, n)
                        first += n

        o_sel = jnp.where(diag, o_sel, 0.0).astype(bf16)
        r0 = pl.multiple_of(hp * R, R)
        return acc + jnp.dot(o_sel, wo_v[pl.ds(r0, R), :], preferred_element_type=f32)

    acc = lax.fori_loop(0, HP, pair_step, jnp.zeros((2 * B, D), f32))
    acc = acc[:B] + acc[B:] + x

    first = 0
    for g, n in enumerate(_W2_GROUPS):
        lo, hi = first * _WO_ROWS, (first + n) * _WO_ROWS
        wait_all(w2_v.at[pl.ds(lo, hi - lo)], w2sem.at[g])
        acc = acc + jnp.dot(hid[:, lo:hi], w2_v[lo:hi, :],
                            preferred_element_type=f32)[:B]
        first += n
    o_ref[...] = acc.astype(o_ref.dtype)


@jax.jit
def pallas_parallel_sum__sliding_block_cached__glu_gated_swiglu__decode_kernel(
    A_x: jax.Array,
    A_k_cache: jax.Array,
    A_v_cache: jax.Array,
    A_wq: jax.Array,
    A_wo: jax.Array,
    B_x: jax.Array,
    B_w1: jax.Array,
    B_w3: jax.Array,
    B_w2: jax.Array,
):
    B, Sq, D = A_x.shape
    _, Hkv, Sk, Dh = A_k_cache.shape
    F = B_w1.shape[1]
    assert Sq == 1 and Hkv == _HQ and Dh == _DH
    assert sum(_W2_GROUPS) * _WO_ROWS == F
    W = min(4096, max(256, Sk // 4))
    bf16 = jnp.bfloat16

    kt = jnp.swapaxes(A_k_cache, 2, 3).reshape(B * Hkv * Dh, Sk)
    vt = jnp.swapaxes(A_v_cache, 2, 3).reshape(B * Hkv * Dh, Sk)
    x2 = A_x.reshape(B, D)

    any_spec = pl.BlockSpec(memory_space=pl.ANY)
    out = pl.pallas_call(
        functools.partial(_kernel, B=B, D=D, F=F, Sk=Sk, W=W),
        in_specs=[any_spec] * 8,
        out_specs=pl.BlockSpec(memory_space=pltpu.VMEM),
        out_shape=jax.ShapeDtypeStruct((B, D), A_x.dtype),
        scratch_shapes=[
            pltpu.VMEM((B, D), bf16),
            pltpu.VMEM(A_wq.shape, bf16),
            pltpu.VMEM(A_wo.shape, bf16),
            pltpu.VMEM(B_w1.shape, bf16),
            pltpu.VMEM(B_w3.shape, bf16),
            pltpu.VMEM(B_w2.shape, bf16),
            pltpu.VMEM((B, W // _LANES, 2 * _DH, _LANES), bf16),
            pltpu.VMEM((B, W // _LANES, 2 * _DH, _LANES), bf16),
            pltpu.VMEM((_HQ // 2, 2 * B, 2 * _DH), jnp.float32),
            pltpu.SemaphoreType.DMA((5,)),
            pltpu.SemaphoreType.DMA((len(_W2_GROUPS),)),
            pltpu.SemaphoreType.DMA((B,)),
            pltpu.SemaphoreType.DMA((B,)),
        ],
        compiler_params=pltpu.CompilerParams(vmem_limit_bytes=100 * 1024 * 1024),
    )(x2, kt, vt, A_wq, A_wo, B_w1, B_w3, B_w2)
    return out.reshape(B, Sq, D)
```

```python
import functools

import jax
import jax.numpy as jnp
from jax import lax
import jax.experimental.pallas as pl
import jax.experimental.pallas.tpu as pltpu

_HQ = 32
_DH = 192
_EPS = 1e-5
_TR = 8
_W2_GROUPS = (20, 16, 8, 4)
_WO_ROWS = 32
_W1_ROWS = 8
_BOUNDS = True
_NSLOT = 2
_COMPUTE = True


def _kernel(x_hbm, k_hbm, v_hbm, wq_hbm, wo_hbm, w1_hbm, w3_hbm, w2_hbm,
            o_ref,
            x_v, wq_v, wo_v, w1_v, w3_v, w2_v, kbuf, vbuf, q_s, o_s, acc_s,
            wsem, w2sem, ksem, vsem,
            *, B, D, F, Sk, W):
    H, Dh = _HQ, _DH
    HP = H // 2
    R = 2 * Dh
    NT = R // _TR
    U = HP * B
    f32, bf16 = jnp.float32, jnp.bfloat16
    scale = Dh ** -0.5

    def start_unit(u):
        slot = u % _NSLOT
        r0 = ((u % B) * HP + u // B) * R

        def body(i, carry):
            ik = i * _TR
            iv = ((i + 4) % 8) * _TR
            for j in range(NT // 8):
                rk = pl.multiple_of(ik + j * 8 * _TR, _TR)
                rv = pl.multiple_of(iv + j * 8 * _TR, _TR)
                pltpu.make_async_copy(
                    k_hbm.at[pl.ds(pl.multiple_of(r0 + rk, _TR), _TR), pl.ds(Sk - W, W)],
                    kbuf.at[slot, pl.ds(rk, _TR)], ksem.at[slot]).start(priority=0)
                pltpu.make_async_copy(
                    v_hbm.at[pl.ds(pl.multiple_of(r0 + rv, _TR), _TR), pl.ds(Sk - W, W)],
                    vbuf.at[slot, pl.ds(rv, _TR)], vsem.at[slot]).start(priority=1)
            return carry
        lax.fori_loop(0, 8, body, 0)

    def wait_all(buf, sem):
        pltpu.make_async_copy(buf, buf, sem).wait()

    def start_chunks(src, dst, sem, rows, cols, first, count, stride):
        n_c = src.shape[1] // cols

        def body(i, a):
            for p in range(2):
                g = first + a
                if n_c == 1:
                    idx = (pl.ds(pl.multiple_of(g * rows, _TR), rows),)
                else:
                    idx = (pl.ds(pl.multiple_of((g // n_c) * rows, _TR), rows),
                           pl.ds(pl.multiple_of((g % n_c) * cols, 128), cols))
                pltpu.make_async_copy(src.at[idx], dst.at[idx], sem).start(priority=p)
                a = a + stride
                a = jnp.where(a >= count, a - count, a)
            return a
        lax.fori_loop(0, count // 2, body, 0)

    x_cp = pltpu.make_async_copy(x_hbm, x_v, wsem.at[0])
    x_cp.start()
    start_chunks(w1_hbm, w1_v, wsem.at[3], _W1_ROWS, F, 0, D // _W1_ROWS, 27)
    start_chunks(w3_hbm, w3_v, wsem.at[4], _W1_ROWS, F, 0, D // _W1_ROWS, 27)
    start_chunks(wq_hbm, wq_v, wsem.at[1], 8, 2048, 0, 240, 23)

    x_cp.wait()
    x = x_v[...].astype(f32)
    mu = jnp.mean(x, axis=-1, keepdims=True)
    xc = x - mu
    var = jnp.mean(xc * xc, axis=-1, keepdims=True)
    xn = xc / jnp.sqrt(var + _EPS)
    xn2 = jnp.concatenate([xn, xn], axis=0).astype(bf16)

    wait_all(w1_v, wsem.at[3])
    wait_all(w3_v, wsem.at[4])
    if _COMPUTE:
        gate = jnp.dot(xn2, w1_v[...], preferred_element_type=f32)
        up = jnp.dot(xn2, w3_v[...], preferred_element_type=f32)
        hid = (gate * jax.nn.sigmoid(gate) * up).astype(bf16)

    start_chunks(wo_hbm, wo_v, wsem.at[2], _WO_ROWS, D, 0, H * Dh // _WO_ROWS, 17)
    lax.fori_loop(0, _NSLOT, lambda u, c: (start_unit(u), c)[1], 0)
    wait_all(wq_v, wsem.at[1])
    wait_all(wo_v, wsem.at[2])

    row = lax.broadcasted_iota(jnp.int32, (2 * B, R), 0)
    col = lax.broadcasted_iota(jnp.int32, (2 * B, R), 1)
    diag = (row >= B) == (col >= Dh)
    row_b = jnp.where(row >= B, row - B, row)
    acc_s[...] = jnp.zeros_like(acc_s)
    o_s[...] = jnp.zeros_like(o_s)

    def unit_step(u, carry):
        slot = u % _NSLOT
        b = u % B
        r0 = pl.multiple_of((u // B) * R, R)

        if _COMPUTE:
            @pl.when(b == 0)
            def _():
                q = jnp.dot(xn2, wq_v[:, pl.ds(r0, R)], preferred_element_type=f32)
                q_s[...] = jnp.where(diag, q, 0.0)

        wait_all(kbuf.at[slot], ksem.at[slot])
        if _COMPUTE:
            s = jnp.dot(q_s[...].astype(bf16), kbuf[slot],
                        preferred_element_type=f32) * scale
            m = jnp.max(s, axis=-1, keepdims=True)
            p = jnp.exp(s - m).astype(bf16)
            l = jnp.sum(p.astype(f32), axis=-1, keepdims=True)
        wait_all(vbuf.at[slot], vsem.at[slot])
        if _COMPUTE:
            o = lax.dot_general(p, vbuf[slot], (((1,), (1,)), ((), ())),
                                preferred_element_type=f32)
            o_s[...] = jnp.where(row_b == b, o / l, o_s[...])

        @pl.when(u + _NSLOT < U)
        def _():
            start_unit(u + _NSLOT)

        @pl.when(u + _NSLOT == U)
        def _():
            first = 0
            for g, n in enumerate(_W2_GROUPS):
                start_chunks(w2_hbm, w2_v, w2sem.at[g], _WO_ROWS, D, first, n,
                             7 if n > 8 else 3)
                first += n

        if _COMPUTE:
            @pl.when(b == B - 1)
            def _():
                o2 = jnp.where(diag, o_s[...], 0.0).astype(bf16)
                acc_s[...] += jnp.dot(o2, wo_v[pl.ds(r0, R), :], preferred_element_type=f32)

        return carry

    lax.fori_loop(0, U, unit_step, 0)
    acc = acc_s[...]
    acc = acc[:B] + acc[B:] + x

    first = 0
    for g, n in enumerate(_W2_GROUPS):
        lo, hi = first * _WO_ROWS, (first + n) * _WO_ROWS
        wait_all(w2_v.at[pl.ds(lo, hi - lo)], w2sem.at[g])
        if _COMPUTE:
            acc = acc + jnp.dot(hid[:, lo:hi], w2_v[lo:hi, :],
                                preferred_element_type=f32)[:B]
        first += n
    o_ref[...] = acc.astype(o_ref.dtype)


@jax.jit
def pallas_parallel_sum__sliding_block_cached__glu_gated_swiglu__decode_kernel(
    A_x: jax.Array,
    A_k_cache: jax.Array,
    A_v_cache: jax.Array,
    A_wq: jax.Array,
    A_wo: jax.Array,
    B_x: jax.Array,
    B_w1: jax.Array,
    B_w3: jax.Array,
    B_w2: jax.Array,
):
    B, Sq, D = A_x.shape
    _, Hkv, Sk, Dh = A_k_cache.shape
    F = B_w1.shape[1]
    assert Sq == 1 and Hkv == _HQ and Dh == _DH
    assert sum(_W2_GROUPS) * _WO_ROWS == F
    W = min(4096, max(256, Sk // 4))
    bf16 = jnp.bfloat16

    kt = jnp.swapaxes(A_k_cache, 2, 3).reshape(B * Hkv * Dh, Sk)
    vt = jnp.swapaxes(A_v_cache, 2, 3).reshape(B * Hkv * Dh, Sk)
    x2 = A_x.reshape(B, D)

    any_spec = pl.BlockSpec(memory_space=pl.ANY)
    out = pl.pallas_call(
        functools.partial(_kernel, B=B, D=D, F=F, Sk=Sk, W=W),
        in_specs=[any_spec] * 8,
        out_specs=pl.BlockSpec(memory_space=pltpu.VMEM),
        out_shape=jax.ShapeDtypeStruct((B, D), A_x.dtype),
        scratch_shapes=[
            pltpu.VMEM((B, D), bf16),
            pltpu.VMEM(A_wq.shape, bf16),
            pltpu.VMEM(A_wo.shape, bf16),
            pltpu.VMEM(B_w1.shape, bf16),
            pltpu.VMEM(B_w3.shape, bf16),
            pltpu.VMEM(B_w2.shape, bf16),
            pltpu.VMEM((_NSLOT, 2 * _DH, W), bf16),
            pltpu.VMEM((_NSLOT, 2 * _DH, W), bf16),
            pltpu.VMEM((2 * B, 2 * _DH), jnp.float32),
            pltpu.VMEM((2 * B, 2 * _DH), jnp.float32),
            pltpu.VMEM((2 * B, D), jnp.float32),
            pltpu.SemaphoreType.DMA((5,)),
            pltpu.SemaphoreType.DMA((len(_W2_GROUPS),)),
            pltpu.SemaphoreType.DMA((_NSLOT,)),
            pltpu.SemaphoreType.DMA((_NSLOT,)),
        ],
        compiler_params=pltpu.CompilerParams(vmem_limit_bytes=64 * 1024 * 1024,
                                             disable_bounds_checks=not _BOUNDS),
    )(x2, kt, vt, A_wq, A_wo, B_w1, B_w3, B_w2)
    return out.reshape(B, Sq, D)
```

```python
import functools

import jax
import jax.numpy as jnp
from jax import lax
import jax.experimental.pallas as pl
import jax.experimental.pallas.tpu as pltpu

_HQ = 32
_DH = 192
_EPS = 1e-5
_TR = 8
_W2_ROWS = 16
_W2_GROUPS = (64, 24, 8)
_W2_STRIDES = (13, 5, 3)
_WO_ROWS = 32
_W1_ROWS = 8
_BOUNDS = True
_SEMCHK = False
_KSLOT = 2
_VSLOT = 4
_VLEAD = 4
_W2_AT = 2
_COMPUTE = True
_JK = (0, 3, 4, 1, 2, 5)
_JV = (0, 3, 4, 1, 2, 5)
_WRR = True
_T1_FIRST = 0
_SCOPES = False


class _NoScope:
    def __enter__(self):
        return self

    def __exit__(self, *a):
        return False


def _scope(name):
    return jax.named_scope(name) if _SCOPES else _NoScope()


def _kernel(x_hbm, k_hbm, v_hbm, wq_hbm, wo_hbm, w1_hbm, w3_hbm, w2_hbm,
            o_ref,
            x_v, wq_v, wo_v, w1_v, w3_v, w2_v, kbuf, vbuf, q_s, o_s, acc_s,
            wsem, w2sem, ksem, vsem,
            *, B, D, F, Sk, W):
    H, Dh = _HQ, _DH
    HP = H // 2
    R = 2 * Dh
    NT = R // _TR
    NG = 8
    GS = NT // NG
    U = HP * B
    f32, bf16 = jnp.float32, jnp.bfloat16
    scale = Dh ** -0.5

    def mult(i):
        return i if isinstance(i, int) else pl.multiple_of(i, _TR)

    def group_copies(src, dst, sem, nslot, g):
        u = g // NG
        slot = u % nslot
        r_in = (g % NG) * _TR
        r0 = ((u % B) * HP + u // B) * R + r_in
        return [pltpu.make_async_copy(
            src.at[pl.ds(mult(r0 + j * NG * _TR), _TR), pl.ds(Sk - W, W)],
            dst.at[slot, pl.ds(mult(r_in + j * NG * _TR), _TR)],
            sem.at[slot]) for j in (_JK if src is k_hbm else _JV)]

    def start_kv(g0, n):
        def body(g, carry):
            for kc, vc in zip(group_copies(k_hbm, kbuf, ksem, _KSLOT, g),
                              group_copies(v_hbm, vbuf, vsem, _VSLOT, g + _VLEAD)):
                kc.start(priority=0)
                vc.start(priority=1)
            return carry
        lax.fori_loop(g0, g0 + n, body, 0)

    def start_single(src, dst, sem, nslot, g0, n, prio):
        def body(g, carry):
            for j, c in enumerate(group_copies(src, dst, sem, nslot, g)):
                c.start(priority=j % 2 if prio is None else prio)
            return carry
        if n:
            lax.fori_loop(g0, g0 + n, body, 0)

    def wait_all(buf, sem):
        pltpu.make_async_copy(buf, buf, sem).wait()

    def start_chunks(src, dst, sem, rows, cols, first, count, stride):
        n_c = src.shape[1] // cols

        def body(i, a):
            for p in range(2):
                g = first + a
                if n_c == 1:
                    idx = (pl.ds(pl.multiple_of(g * rows, _TR), rows),)
                else:
                    idx = (pl.ds(pl.multiple_of((g // n_c) * rows, _TR), rows),
                           pl.ds(pl.multiple_of((g % n_c) * cols, 128), cols))
                pltpu.make_async_copy(src.at[idx], dst.at[idx], sem).start(priority=p)
                a = a + stride
                a = jnp.where(a >= count, a - count, a)
            return a
        lax.fori_loop(0, count // 2, body, 0)

    n_w2 = F // _W2_ROWS
    n_lead = _VLEAD * GS
    n_t0 = (n_w2 - n_lead) // 2
    w2_seq, first = [], 0
    for g, n in enumerate(_W2_GROUPS):
        w2_seq += [(g, first + (i * _W2_STRIDES[g]) % n) for i in range(n)]
        first += n
    n_mix = _W2_GROUPS[0] - n_t0
    n_pre = n_t0 - n_mix
    w2_t0 = w2_seq[:n_pre] + w2_seq[n_pre:_W2_GROUPS[0]:2]
    w2_t1 = w2_seq[n_pre + 1:_W2_GROUPS[0]:2] + w2_seq[_W2_GROUPS[0]:]
    assert len(w2_t0) == n_t0 and len(w2_t1) == n_w2 - n_t0

    def w2_copy(g, c):
        rows = pl.ds(c * _W2_ROWS, _W2_ROWS)
        return pltpu.make_async_copy(w2_hbm.at[rows], w2_v.at[rows], w2sem.at[g])

    x_cp = pltpu.make_async_copy(x_hbm, x_v, wsem.at[0])
    x_cp.start()
    if _WRR:
        n_it = 4
        wq_tr, wo_tr, w1_tr = D // _TR, H * Dh // _TR, D // _TR
        wo_cuts = [(16 * i + 2) // 5 for i in range(16)]
        assert wo_cuts[-1] * 4 * n_it == wo_tr

        def w_body(it, carry):
            def rows(t, n):
                return pl.ds(pl.multiple_of(t * _TR, _TR), n * _TR)

            def wq_c(k, i):
                idx = (rows(k * (wq_tr // 4) + it * (wq_tr // 4 // n_it) + i // 3, 1),
                       pl.ds((i % 3) * 2048, 2048))
                return pltpu.make_async_copy(wq_hbm.at[idx], wq_v.at[idx], wsem.at[1])

            def wo_c(k, i):
                idx = rows(k * (wo_tr // 4) + it * wo_cuts[-1] + wo_cuts[i],
                           wo_cuts[i + 1] - wo_cuts[i])
                return pltpu.make_async_copy(wo_hbm.at[idx], wo_v.at[idx], wsem.at[2])

            def w13_c(k, i):
                idx = rows(it * (w1_tr // n_it) + i, 1)
                src, dst = ((w1_hbm, w1_v), (w3_hbm, w3_v))[k]
                return pltpu.make_async_copy(src.at[idx], dst.at[idx], wsem.at[3 + k])

            seq = []
            for r in range(w1_tr // n_it):
                big = (r + 1) * 3 // 4 > r * 3 // 4
                for k in range(4):
                    if big:
                        seq += [wq_c(k, r * 3 // 4), wo_c(k, r * 3 // 4)]
                    if k % 2 == 0:
                        seq.append(w13_c(k // 2, r))
            for i, c in enumerate(seq):
                c.start(priority=i % 2)
            return carry
        lax.fori_loop(0, n_it, w_body, 0)
        start_single(v_hbm, vbuf, vsem, _VSLOT, 0, _VLEAD, None)
        start_kv(0, NG)
    else:
        start_chunks(w1_hbm, w1_v, wsem.at[3], _W1_ROWS, F, 0, D // _W1_ROWS, 27)
        start_chunks(w3_hbm, w3_v, wsem.at[4], _W1_ROWS, F, 0, D // _W1_ROWS, 27)
        start_chunks(wq_hbm, wq_v, wsem.at[1], 8, 2048, 0, 240, 23)

    x_cp.wait()
    x = x_v[...].astype(f32)
    mu = jnp.mean(x, axis=-1, keepdims=True)
    xc = x - mu
    var = jnp.mean(xc * xc, axis=-1, keepdims=True)
    xn = xc / jnp.sqrt(var + _EPS)
    xn2 = jnp.concatenate([xn, xn], axis=0).astype(bf16)

    wait_all(w1_v, wsem.at[3])
    wait_all(w3_v, wsem.at[4])
    if _COMPUTE:
        gate = jnp.dot(xn2, w1_v[...], preferred_element_type=f32)
        up = jnp.dot(xn2, w3_v[...], preferred_element_type=f32)
        hid = (gate * jax.nn.sigmoid(gate) * up).astype(bf16)

    if _WRR:
        start_kv(NG, (_KSLOT - 1) * NG)
    else:
        start_chunks(wo_hbm, wo_v, wsem.at[2], _WO_ROWS, D, 0, H * Dh // _WO_ROWS, 17)
        start_single(v_hbm, vbuf, vsem, _VSLOT, 0, _VLEAD, None)
        start_kv(0, _KSLOT * NG)
    wait_all(wq_v, wsem.at[1])
    wait_all(wo_v, wsem.at[2])

    row = lax.broadcasted_iota(jnp.int32, (2 * B, R), 0)
    col = lax.broadcasted_iota(jnp.int32, (2 * B, R), 1)
    diag = (row >= B) == (col >= Dh)
    row_b = jnp.where(row >= B, row - B, row)
    acc_s[...] = jnp.zeros_like(acc_s)
    o_s[...] = jnp.zeros_like(o_s)

    def unit_step(u, carry):
        kslot = u % _KSLOT
        vslot = u % _VSLOT
        b = u % B
        r0 = pl.multiple_of((u // B) * R, R)

        if _COMPUTE:
            @pl.when(b == 0)
            def _():
                q = jnp.dot(xn2, wq_v[:, pl.ds(r0, R)], preferred_element_type=f32)
                q_s[...] = jnp.where(diag, q, 0.0)

        with _scope("kwait"):
            wait_all(kbuf.at[kslot], ksem.at[kslot])
        if _COMPUTE:
            s = jnp.dot(q_s[...].astype(bf16), kbuf[kslot],
                        preferred_element_type=f32) * scale
            m = jnp.max(s, axis=-1, keepdims=True)
            p = jnp.exp(s - m).astype(bf16)
            l = jnp.sum(p.astype(f32), axis=-1, keepdims=True)
        with _scope("vwait"):
            wait_all(vbuf.at[vslot], vsem.at[vslot])
        if _COMPUTE:
            o = lax.dot_general(p, vbuf[vslot], (((1,), (1,)), ((), ())),
                                preferred_element_type=f32)
            o_s[...] = jnp.where(row_b == b, o / l, o_s[...])

        with _scope("issue"):
            g0 = (u + _KSLOT) * NG
            n_pair = jnp.clip(U * NG - _VLEAD - g0, 0, NG)
            start_kv(g0, n_pair)

            @pl.when(u + _KSLOT == U - 1)
            def _():
                kcs = [c for g in range(U * NG - _VLEAD, U * NG)
                       for c in group_copies(k_hbm, kbuf, ksem, _KSLOT, g)]
                for kc, w in zip(kcs, w2_t1[:n_lead]):
                    kc.start(priority=0)
                    w2_copy(*w).start(priority=1)

            @pl.when(u == U - _W2_AT)
            def _():
                for w0, w1 in zip(w2_t0, w2_t1[n_lead:]):
                    w2_copy(*w0).start(priority=0)
                    w2_copy(*w1).start(priority=1)

        if _COMPUTE:
            @pl.when(b == B - 1)
            def _():
                with _scope("womm"):
                    o2 = jnp.where(diag, o_s[...], 0.0).astype(bf16)
                    acc_s[...] += jnp.dot(o2, wo_v[pl.ds(r0, R), :], preferred_element_type=f32)

        return carry

    lax.fori_loop(0, U, unit_step, 0)
    acc = acc_s[...]
    acc = acc[:B] + acc[B:] + x

    first = 0
    for g, n in enumerate(_W2_GROUPS):
        lo, hi = first * _W2_ROWS, (first + n) * _W2_ROWS
        with _scope(f"w2wait{g}"):
            wait_all(w2_v.at[pl.ds(lo, hi - lo)], w2sem.at[g])
        if _COMPUTE:
            with _scope(f"w2mm{g}"):
                acc = acc + jnp.dot(hid[:, lo:hi], w2_v[lo:hi, :],
                                    preferred_element_type=f32)[:B]
        first += n
    o_ref[...] = acc.astype(o_ref.dtype)


@jax.jit
def pallas_parallel_sum__sliding_block_cached__glu_gated_swiglu__decode_kernel(
    A_x: jax.Array,
    A_k_cache: jax.Array,
    A_v_cache: jax.Array,
    A_wq: jax.Array,
    A_wo: jax.Array,
    B_x: jax.Array,
    B_w1: jax.Array,
    B_w3: jax.Array,
    B_w2: jax.Array,
):
    B, Sq, D = A_x.shape
    _, Hkv, Sk, Dh = A_k_cache.shape
    F = B_w1.shape[1]
    assert Sq == 1 and Hkv == _HQ and Dh == _DH
    assert sum(_W2_GROUPS) * _W2_ROWS == F
    W = min(4096, max(256, Sk // 4))
    bf16 = jnp.bfloat16

    kt = jnp.swapaxes(A_k_cache, 2, 3).reshape(B * Hkv * Dh, Sk)
    vt = jnp.swapaxes(A_v_cache, 2, 3).reshape(B * Hkv * Dh, Sk)
    x2 = A_x.reshape(B, D)

    any_spec = pl.BlockSpec(memory_space=pl.ANY)
    out = pl.pallas_call(
        functools.partial(_kernel, B=B, D=D, F=F, Sk=Sk, W=W),
        in_specs=[any_spec] * 8,
        out_specs=pl.BlockSpec(memory_space=pltpu.VMEM),
        out_shape=jax.ShapeDtypeStruct((B, D), A_x.dtype),
        scratch_shapes=[
            pltpu.VMEM((B, D), bf16),
            pltpu.VMEM(A_wq.shape, bf16),
            pltpu.VMEM(A_wo.shape, bf16),
            pltpu.VMEM(B_w1.shape, bf16),
            pltpu.VMEM(B_w3.shape, bf16),
            pltpu.VMEM(B_w2.shape, bf16),
            pltpu.VMEM((_KSLOT, 2 * _DH, W), bf16),
            pltpu.VMEM((_VSLOT, 2 * _DH, W), bf16),
            pltpu.VMEM((2 * B, 2 * _DH), jnp.float32),
            pltpu.VMEM((2 * B, 2 * _DH), jnp.float32),
            pltpu.VMEM((2 * B, D), jnp.float32),
            pltpu.SemaphoreType.DMA((5,)),
            pltpu.SemaphoreType.DMA((len(_W2_GROUPS),)),
            pltpu.SemaphoreType.DMA((_KSLOT,)),
            pltpu.SemaphoreType.DMA((_VSLOT,)),
        ],
        compiler_params=pltpu.CompilerParams(vmem_limit_bytes=64 * 1024 * 1024,
                                             disable_bounds_checks=not _BOUNDS,
                                             disable_semaphore_checks=not _SEMCHK),
    )(x2, kt, vt, A_wq, A_wo, B_w1, B_w3, B_w2)
    return out.reshape(B, Sq, D)
```

```python
import functools

import jax
import jax.numpy as jnp
from jax import lax
import jax.experimental.pallas as pl
import jax.experimental.pallas.tpu as pltpu

_HQ = 32
_DH = 192
_EPS = 1e-5
_TR = 8
_NG = 8
_JORDER = (0, 3, 4, 1, 2, 5)
_KSLOT = 2
_VSLOT = 4
_VLEAD = 4
_WQ_COLS = 2048
_W2_ROWS = 16
_W2_GROUPS = (64, 24, 8)
_W2_STRIDES = (13, 5, 3)


def _kernel(x_hbm, k_hbm, v_hbm, wq_hbm, wo_hbm, w1_hbm, w3_hbm, w2_hbm,
            o_ref,
            x_v, wq_v, wo_v, w1_v, w3_v, w2_v, kbuf, vbuf, q_s, o_s, acc_s,
            wsem, w2sem, ksem, vsem,
            *, B, D, F, Sk, W):
    H, Dh = _HQ, _DH
    HP = H // 2
    R = 2 * Dh
    U = HP * B
    GS = len(_JORDER)
    assert R == _NG * GS * _TR
    f32, bf16 = jnp.float32, jnp.bfloat16
    scale = Dh ** -0.5

    def tile_rows(t, n=1):
        r = t * _TR
        return pl.ds(r if isinstance(r, int) else pl.multiple_of(r, _TR), n * _TR)

    def wait_all(buf, sem):
        pltpu.make_async_copy(buf, buf, sem).wait()

    def group_copies(src, dst, sem, nslot, g):
        u = g // _NG
        i = g % _NG
        slot = u % nslot
        t0 = ((u % B) * HP + u // B) * (R // _TR) + i
        return [pltpu.make_async_copy(
            src.at[tile_rows(t0 + j * _NG), pl.ds(Sk - W, W)],
            dst.at[slot, tile_rows(i + j * _NG)], sem.at[slot]) for j in _JORDER]

    k_copies = functools.partial(group_copies, k_hbm, kbuf, ksem, _KSLOT)
    v_copies = functools.partial(group_copies, v_hbm, vbuf, vsem, _VSLOT)

    def start_kv(g0, n):
        def body(g, carry):
            for kc, vc in zip(k_copies(g), v_copies(g + _VLEAD)):
                kc.start(priority=0)
                vc.start(priority=1)
            return carry
        lax.fori_loop(g0, g0 + n, body, 0)

    def start_v_lead():
        def body(g, carry):
            for j, vc in enumerate(v_copies(g)):
                vc.start(priority=j % 2)
            return carry
        lax.fori_loop(0, _VLEAD, body, 0)

    def start_weights():
        n_it = 4
        n_qc = H * Dh // _WQ_COLS
        wq_tr, wo_tr, w1_tr = D // _TR, H * Dh // _TR, D // _TR
        n_big = wq_tr * n_qc // 4 // n_it
        n_small = w1_tr // n_it
        wo_step = wo_tr // 4 // n_it
        wo_cuts = [(2 * wo_step * i + n_big) // (2 * n_big) for i in range(n_big + 1)]

        def body(it, carry):
            def wq_copy(k, i):
                idx = (tile_rows(k * (wq_tr // 4) + it * (n_big // n_qc) + i // n_qc),
                       pl.ds((i % n_qc) * _WQ_COLS, _WQ_COLS))
                return pltpu.make_async_copy(wq_hbm.at[idx], wq_v.at[idx], wsem.at[1])

            def wo_copy(k, i):
                idx = tile_rows(k * (wo_tr // 4) + it * wo_step + wo_cuts[i],
                                wo_cuts[i + 1] - wo_cuts[i])
                return pltpu.make_async_copy(wo_hbm.at[idx], wo_v.at[idx], wsem.at[2])

            def w13_copy(k, i):
                idx = tile_rows(it * n_small + i)
                src, dst = ((w1_hbm, w1_v), (w3_hbm, w3_v))[k]
                return pltpu.make_async_copy(src.at[idx], dst.at[idx], wsem.at[3 + k])

            seq = []
            for r in range(n_small):
                i = r * n_big // n_small
                for k in range(4):
                    if (r + 1) * n_big // n_small > i:
                        seq += [wq_copy(k, i), wo_copy(k, i)]
                    if k % 2 == 0:
                        seq.append(w13_copy(k // 2, r))
            assert len(seq) == 8 * n_big + 2 * n_small and len(seq) % 2 == 0
            for n, c in enumerate(seq):
                c.start(priority=n % 2)
            return carry
        lax.fori_loop(0, n_it, body, 0)

    n_w2 = F // _W2_ROWS
    n_lead = _VLEAD * GS
    n_q0 = (n_w2 - n_lead) // 2
    w2_seq, first = [], 0
    for g, n in enumerate(_W2_GROUPS):
        w2_seq += [(g, first + (i * _W2_STRIDES[g]) % n) for i in range(n)]
        first += n
    n_pre = 2 * n_q0 - _W2_GROUPS[0]
    w2_q0 = w2_seq[:n_pre] + w2_seq[n_pre:_W2_GROUPS[0]:2]
    w2_q1 = w2_seq[n_pre + 1:_W2_GROUPS[0]:2] + w2_seq[_W2_GROUPS[0]:]
    assert sorted(c for _, c in w2_q0 + w2_q1) == list(range(n_w2))
    assert len(w2_q0) == n_q0 and len(w2_q1) == n_lead + n_q0

    def w2_copy(g, c):
        rows = pl.ds(c * _W2_ROWS, _W2_ROWS)
        return pltpu.make_async_copy(w2_hbm.at[rows], w2_v.at[rows], w2sem.at[g])

    x_cp = pltpu.make_async_copy(x_hbm, x_v, wsem.at[0])
    x_cp.start()
    start_weights()
    start_v_lead()
    start_kv(0, _NG)

    x_cp.wait()
    x = x_v[...].astype(f32)
    mu = jnp.mean(x, axis=-1, keepdims=True)
    xc = x - mu
    var = jnp.mean(xc * xc, axis=-1, keepdims=True)
    xn = xc / jnp.sqrt(var + _EPS)
    xn2 = jnp.concatenate([xn, xn], axis=0).astype(bf16)

    wait_all(w1_v, wsem.at[3])
    wait_all(w3_v, wsem.at[4])
    gate = jnp.dot(xn2, w1_v[...], preferred_element_type=f32)
    up = jnp.dot(xn2, w3_v[...], preferred_element_type=f32)
    hid = (gate * jax.nn.sigmoid(gate) * up).astype(bf16)

    start_kv(_NG, (_KSLOT - 1) * _NG)
    wait_all(wq_v, wsem.at[1])
    wait_all(wo_v, wsem.at[2])

    row = lax.broadcasted_iota(jnp.int32, (2 * B, R), 0)
    col = lax.broadcasted_iota(jnp.int32, (2 * B, R), 1)
    diag = (row >= B) == (col >= Dh)
    row_b = jnp.where(row >= B, row - B, row)
    acc_s[...] = jnp.zeros_like(acc_s)
    o_s[...] = jnp.zeros_like(o_s)

    def unit_step(u, carry):
        kslot = u % _KSLOT
        vslot = u % _VSLOT
        b = u % B
        r0 = pl.multiple_of((u // B) * R, R)

        @pl.when(b == 0)
        def _():
            q = jnp.dot(xn2, wq_v[:, pl.ds(r0, R)], preferred_element_type=f32)
            q_s[...] = jnp.where(diag, q, 0.0)

        wait_all(kbuf.at[kslot], ksem.at[kslot])
        s = jnp.dot(q_s[...].astype(bf16), kbuf[kslot],
                    preferred_element_type=f32) * scale
        m = jnp.max(s, axis=-1, keepdims=True)
        p = jnp.exp(s - m).astype(bf16)
        l = jnp.sum(p.astype(f32), axis=-1, keepdims=True)
        wait_all(vbuf.at[vslot], vsem.at[vslot])
        o = lax.dot_general(p, vbuf[vslot], (((1,), (1,)), ((), ())),
                            preferred_element_type=f32)
        o_s[...] = jnp.where(row_b == b, o / l, o_s[...])

        g0 = (u + _KSLOT) * _NG
        start_kv(g0, jnp.clip(U * _NG - _VLEAD - g0, 0, _NG))

        @pl.when(u + _KSLOT == U - 1)
        def _():
            kcs = [c for g in range(U * _NG - _VLEAD, U * _NG) for c in k_copies(g)]
            for kc, w in zip(kcs, w2_q1[:n_lead]):
                kc.start(priority=0)
                w2_copy(*w).start(priority=1)

        @pl.when(u + _KSLOT == U)
        def _():
            for w0, w1 in zip(w2_q0, w2_q1[n_lead:]):
                w2_copy(*w0).start(priority=0)
                w2_copy(*w1).start(priority=1)

        @pl.when(b == B - 1)
        def _():
            o2 = jnp.where(diag, o_s[...], 0.0).astype(bf16)
            acc_s[...] += jnp.dot(o2, wo_v[pl.ds(r0, R), :], preferred_element_type=f32)

        return carry

    lax.fori_loop(0, U, unit_step, 0)
    acc = acc_s[...]
    acc = acc[:B] + acc[B:] + x

    first = 0
    for g, n in enumerate(_W2_GROUPS):
        lo, hi = first * _W2_ROWS, (first + n) * _W2_ROWS
        wait_all(w2_v.at[pl.ds(lo, hi - lo)], w2sem.at[g])
        acc = acc + jnp.dot(hid[:, lo:hi], w2_v[lo:hi, :],
                            preferred_element_type=f32)[:B]
        first += n
    o_ref[...] = acc.astype(o_ref.dtype)


@jax.jit
def pallas_parallel_sum__sliding_block_cached__glu_gated_swiglu__decode_kernel(
    A_x: jax.Array,
    A_k_cache: jax.Array,
    A_v_cache: jax.Array,
    A_wq: jax.Array,
    A_wo: jax.Array,
    B_x: jax.Array,
    B_w1: jax.Array,
    B_w3: jax.Array,
    B_w2: jax.Array,
):
    del B_x
    B, Sq, D = A_x.shape
    _, Hkv, Sk, Dh = A_k_cache.shape
    F = B_w1.shape[1]
    assert Sq == 1 and Hkv == _HQ and Dh == _DH
    assert sum(_W2_GROUPS) * _W2_ROWS == F
    W = min(4096, max(256, Sk // 4))
    bf16, f32 = jnp.bfloat16, jnp.float32

    kt = jnp.swapaxes(A_k_cache, 2, 3).reshape(B * Hkv * Dh, Sk)
    vt = jnp.swapaxes(A_v_cache, 2, 3).reshape(B * Hkv * Dh, Sk)

    out = pl.pallas_call(
        functools.partial(_kernel, B=B, D=D, F=F, Sk=Sk, W=W),
        in_specs=[pl.BlockSpec(memory_space=pl.ANY)] * 8,
        out_specs=pl.BlockSpec(memory_space=pltpu.VMEM),
        out_shape=jax.ShapeDtypeStruct((B, D), A_x.dtype),
        scratch_shapes=[
            pltpu.VMEM((B, D), bf16),
            pltpu.VMEM(A_wq.shape, bf16),
            pltpu.VMEM(A_wo.shape, bf16),
            pltpu.VMEM(B_w1.shape, bf16),
            pltpu.VMEM(B_w3.shape, bf16),
            pltpu.VMEM(B_w2.shape, bf16),
            pltpu.VMEM((_KSLOT, 2 * _DH, W), bf16),
            pltpu.VMEM((_VSLOT, 2 * _DH, W), bf16),
            pltpu.VMEM((2 * B, 2 * _DH), f32),
            pltpu.VMEM((2 * B, 2 * _DH), f32),
            pltpu.VMEM((2 * B, D), f32),
            pltpu.SemaphoreType.DMA((5,)),
            pltpu.SemaphoreType.DMA((len(_W2_GROUPS),)),
            pltpu.SemaphoreType.DMA((_KSLOT,)),
            pltpu.SemaphoreType.DMA((_VSLOT,)),
        ],
        compiler_params=pltpu.CompilerParams(
            vmem_limit_bytes=64 * 1024 * 1024,
            disable_semaphore_checks=True,
        ),
    )(A_x.reshape(B, D), kt, vt, A_wq, A_wo, B_w1, B_w3, B_w2)
    return out.reshape(B, Sq, D)
```
